```python
import os as _os
_os.environ.setdefault('JAX_PLATFORMS', 'cpu')
import jax
import jax.numpy as jnp

def _softmax(x, axis=-1):
    return jax.nn.softmax(x, axis=axis)

def _gelu(x):
    return jax.nn.gelu(x, approximate=True)

def _silu(x):
    return jax.nn.silu(x)

def _sigmoid(x):
    return jax.nn.sigmoid(x)

def _layernorm(x, axis=-1, eps=1e-05):
    m = jnp.mean(x, axis=axis, keepdims=True)
    v = jnp.var(x, axis=axis, keepdims=True)
    return (x - m) / jnp.sqrt(v + eps)

def _scatter_add(tgt, idx, src, axis=0):
    return tgt.at[idx].add(src)

def _segment_sum(src, seg, n):
    return jax.ops.segment_sum(src, seg, n)

class _Rng:

    def __init__(self, key):
        self._k = key

    def _next(self):
        self._k, sub = jax.random.split(self._k)
        return sub

    def normal(self, shape):
        return jax.random.normal(self._next(), shape, dtype=jnp.bfloat16)

    def randint(self, lo, hi, shape):
        return jax.random.randint(self._next(), shape, lo, hi, dtype=jnp.int32)

    def uniform(self, shape, lo=0.0, hi=1.0):
        return jax.random.uniform(self._next(), shape, jnp.bfloat16, lo, hi)

    def permutation(self, n):
        return jax.random.permutation(self._next(), n)
kernel_name = 'adaLN_cond__memory_aug_recurrent_mem_tr__moe_arch_mod__prompt'

def setup_inputs():
    _rng = _Rng(jax.random.key(int.from_bytes(__import__("os").urandom(4), "little")))
    _w = lambda a: (lambda t: t.astype(jnp.bfloat16) if jnp.issubdtype(t.dtype, jnp.floating) else t)(jnp.asarray(a))

    def _A_setup():
        B, S, Dm = (1, 2048, 448)
        H, Dh = (16, 256)
        M, seg = (8, 32)
        seg = min(seg, S)
        S = S // seg * seg
        return {'x': _w((lambda *s: _rng.normal(s) * 0.05)(B, S, Dm)), 'mem0': _w((lambda *s: _rng.normal(s) * 0.4)(B, M, Dm)), 'Wq': _w((lambda *s: _rng.normal(s) * 1.6)(Dm, H, Dh) * Dm ** (-0.5)), 'Wk': _w((lambda *s: _rng.normal(s) * 1.6)(Dm, H, Dh) * Dm ** (-0.5)), 'Wv': _w((lambda *s: _rng.normal(s) * 0.4)(Dm, H, Dh) * Dm ** (-0.5)), 'Wo': _w((lambda *s: _rng.normal(s) * 0.4)(H, Dh, Dm) * (H * Dh) ** (-0.5)), 'seg_len': seg}
    _A_in = _A_setup()

    def _B_setup():
        B, S, D, F, C = (1, 2048, 448, 1792, 1)
        return {'x': _w((lambda *s: _rng.normal(s) * 0.05)(B, S, D)), 'w_r': _w((lambda *s: _rng.normal(s) * 0.05)(D)), 'w_gate': _w((lambda *s: _rng.normal(s) * 0.05)(D, F)), 'w_up': _w((lambda *s: _rng.normal(s) * 0.05)(D, F)), 'w_down': _w((lambda *s: _rng.normal(s) * 0.05)(F, D))}
    _B_in = _B_setup()
    return {'A_x': _A_in['x'], 'A_mem0': _A_in['mem0'], 'A_Wq': _A_in['Wq'], 'A_Wk': _A_in['Wk'], 'A_Wv': _A_in['Wv'], 'A_Wo': _A_in['Wo'], 'A_seg_len': _A_in['seg_len'], 'B_x': _B_in['x'], 'B_w_r': _B_in['w_r'], 'B_w_gate': _B_in['w_gate'], 'B_w_up': _B_in['w_up'], 'B_w_down': _B_in['w_down'], 'c': _w((lambda *s: _rng.normal(s) * 0.05)(1, 448) * 8.0), 'w_mod': _w((lambda *s: _rng.normal(s) * 0.05)(448, 6 * 448) * 448 ** (-0.5) * 8.0)}

def reference(A_x, A_mem0, A_Wq, A_Wk, A_Wv, A_Wo, A_seg_len, B_x, B_w_r, B_w_gate, B_w_up, B_w_down, c, w_mod):

    def _A_ref(x, mem0, Wq, Wk, Wv, Wo, seg_len):
        B, S, Dm = x.shape
        H, Dh = (Wq.shape[1], Wq.shape[2])
        M = mem0.shape[1]
        scale = Dh ** (-0.5)
        n_seg = S // seg_len
        L = M + seg_len
        idx = jnp.arange(L)
        mask = (idx[:, None] < M) | (idx[:, None] >= idx[None, :])
        mem = mem0
        outs = []
        for s in range(n_seg):
            xs = x[:, s * seg_len:(s + 1) * seg_len, :].copy()
            h = jnp.concatenate([mem, xs], axis=1)
            q = jnp.einsum('btd,dhe->bhte', h, Wq)
            k = jnp.einsum('btd,dhe->bhte', h, Wk)
            v = jnp.einsum('btd,dhe->bhte', h, Wv)
            scores = jnp.einsum('bhqe,bhke->bhqk', q, k) * scale
            scores = jnp.where(mask[None, None], scores, -1000000000.0)
            p = _softmax(scores, axis=-1)
            o = jnp.einsum('bhqk,bhke->bhqe', p, v)
            o = jnp.einsum('bhte,hed->btd', o, Wo)
            mem = o[:, :M, :].copy()
            outs.append(o[:, M:, :])
        return jnp.concatenate(outs, axis=1)

    def _B_ref(x, w_r, w_gate, w_up, w_down):
        B, S, D = x.shape
        C = 1
        r = x @ w_r
        idx = jnp.argsort(-r, axis=-1)[:, :C]
        idx_e = jnp.repeat(idx.reshape(B, C, 1), D, axis=2)
        x_sel = jnp.take_along_axis(x, idx_e, axis=1)
        g = _silu(x_sel @ w_gate)
        u = x_sel @ w_up
        y = g * u @ w_down
        r_sel = _sigmoid(jnp.take_along_axis(r, idx, axis=1))
        y = y * r_sel.reshape(B, C, 1)
        b_off = (jnp.arange(B) * S).reshape(B, 1)
        flat_idx = (idx + b_off).reshape(B * C)
        zero = (x * 0.0).reshape(B * S, D)
        upd = _scatter_add(zero, flat_idx, y.reshape(B * C, D), axis=0)
        return x + upd.reshape(B, S, D)
    x = A_x
    mod = (_silu(c) @ w_mod).reshape(c.shape[0], 6, 1, -1)
    sa, ca, ga, sb, cb, gb = (mod[:, 0].copy(), mod[:, 1].copy(), mod[:, 2].copy(), mod[:, 3].copy(), mod[:, 4].copy(), mod[:, 5].copy())
    h = _layernorm(x, axis=-1) * (1 + ca) + sa
    x = x + ga * _A_ref(h, A_mem0, A_Wq, A_Wk, A_Wv, A_Wo, A_seg_len)
    h = _layernorm(x, axis=-1) * (1 + cb) + sb
    x = x + gb * _B_ref(h, B_w_r, B_w_gate, B_w_up, B_w_down)
    return x
```

```python
import functools

import jax
import jax.numpy as jnp
from jax import lax
import jax.experimental.pallas as pl
import jax.experimental.pallas.tpu as pltpu

F32 = jnp.float32
BF16 = jnp.bfloat16
U32 = jnp.uint32

_NN = (((1,), (0,)), ((), ()))
_NT = (((1,), (1,)), ((), ()))

LANES = 128


def _dot(a, b, dims):
    return lax.dot_general(a, b, dims, preferred_element_type=F32)


def _rb(x):
    return x.astype(BF16).astype(F32)


def _unpack(w):
    lo = pltpu.bitcast(w << 16, F32)
    hi = pltpu.bitcast(w & jnp.uint32(0xFFFF0000), F32)
    return lo, hi


def _tiles(x):
    return [x[:, t * LANES:(t + 1) * LANES] for t in range(x.shape[1] // LANES)]


def _kernel(xT_hbm, mem0_ref, wq_hbm, wk_hbm, wv_hbm, woT_hbm, wr_ref, wg_hbm, wu_hbm, wdT_hbm,
            c_ref, wmod_hbm, outT_hbm,
            bq, bk, bv, bo, wa, wb, wmod_v, xT_v, xN, hs, h2s, outN, outT_v, wg_v, wu_v, wd_v,
            par, att, sem_w, sem_x, sem_o, sem_m,
            *, S, D, H, E, M, SEG):
    NG = S // LANES
    NSEG = S // SEG
    SPG = LANES // SEG
    L = M + SEG
    NB = L // 8
    NP = H // 2
    FULL = D // LANES
    REM = D - FULL * LANES
    NT = FULL + 1
    scale = float(E) ** -0.5

    wq32 = wq_hbm.bitcast(U32)
    wk32 = wk_hbm.bitcast(U32)
    wv32 = wv_hbm.bitcast(U32)

    def w_copies(i):
        return (
            pltpu.make_async_copy(wq32.at[:, i, :], bq.at[i], sem_w.at[0, i]),
            pltpu.make_async_copy(wk32.at[:, i, :], bk.at[i], sem_w.at[1, i]),
            pltpu.make_async_copy(wv32.at[:, i, :], bv.at[i], sem_w.at[2, i]),
            pltpu.make_async_copy(woT_hbm.at[pl.ds(2 * i, 2)], bo.at[i], sem_w.at[3, i]),
        )

    def x_copy(g):
        return pltpu.make_async_copy(xT_hbm.at[:, g * LANES:(g + 1) * LANES], xT_v.at[g], sem_x.at[g])

    mod_copy = pltpu.make_async_copy(wmod_hbm, wmod_v, sem_m.at[0])
    ffn_copies = (
        pltpu.make_async_copy(wg_hbm, wg_v, sem_m.at[1]),
        pltpu.make_async_copy(wu_hbm, wu_v, sem_m.at[2]),
        pltpu.make_async_copy(wdT_hbm, wd_v, sem_m.at[3]),
    )

    AHEAD = 2
    for i in range(AHEAD):
        for cp in w_copies(i):
            cp.start()

    lane = lax.broadcasted_iota(jnp.int32, (8, LANES), 1)
    sub = lax.broadcasted_iota(jnp.int32, (8, LANES), 0)

    zpad = jnp.zeros((wa.shape[0], (NT * LANES - D) // 2, LANES), U32)
    wa[:, D // 2:, :] = zpad
    wb[:, D // 2:, :] = zpad
    outN[0:LANES, :] = jnp.zeros((LANES, NT * LANES), F32)

    def fuse(lhs_lo, lhs_hi, r_lo, r_hi, dst, i, mul):
        rem = jnp.concatenate([r_lo[FULL * LANES:], r_hi[FULL * LANES:]], axis=0)
        outs = []
        for j, (lhs, r) in enumerate(((lhs_lo, r_lo), (lhs_hi, r_hi))):
            rhs = jnp.concatenate([r[:FULL * LANES], rem], axis=0)
            o = _dot(lhs, rhs, _NT)
            if mul != 1.0:
                o = o * mul
            for t in range(FULL):
                dst[t * H + 2 * i + j, 0:D // 2, :] = pltpu.bitcast(
                    o[:, t * LANES:(t + 1) * LANES].astype(BF16), U32)
            outs.append(o[:, FULL * LANES:])
        low = lax.broadcasted_iota(jnp.int32, (D, LANES), 1) < REM
        dst[FULL * H + i, 0:D // 2, :] = pltpu.bitcast(
            jnp.where(low, outs[0], outs[1]).astype(BF16), U32)

    def pre_body(i, carry):
        for cp in w_copies(i):
            cp.wait()

        @pl.when(i + AHEAD < NP)
        def _():
            for cp in w_copies(i + AHEAD):
                cp.start()

        @pl.when(i + AHEAD == NP)
        def _():
            mod_copy.start()
            x_copy(0).start()

        q_lo, q_hi = _unpack(bq[i])
        k_lo, k_hi = _unpack(bk[i])
        fuse(k_lo, k_hi, q_lo.astype(BF16), q_hi.astype(BF16), wa, i, scale)
        v_lo, v_hi = _unpack(bv[i])
        fuse(v_lo, v_hi, bo[i, 0], bo[i, 1], wb, i, 1.0)
        return carry

    lax.fori_loop(0, NP, pre_body, 0)

    for g in range(1, NG):
        x_copy(g).start()
    for cp in ffn_copies:
        cp.start()

    mod_copy.wait()
    cv = jnp.broadcast_to(c_ref[...].astype(F32), (8, D))
    sc = _rb(cv * jax.nn.sigmoid(cv))
    mod = _rb(_dot(sc.astype(BF16), wmod_v[...], _NN))

    def dup(v):
        return jnp.concatenate([v, v[:, FULL * LANES:]], axis=1)

    for j in range(6):
        v = mod[:, j * D:(j + 1) * D]
        if j in (1, 4):
            v = _rb(1.0 + v)
        par[j] = dup(v)
    wr = jnp.broadcast_to(wr_ref[...].astype(F32).reshape(1, D), (8, D))
    par[6] = jnp.concatenate([wr, jnp.zeros((8, REM), F32)], axis=1)

    def load_x_block(g, k):
        r0 = pl.multiple_of(k * LANES, REM)
        r1 = pl.multiple_of(jnp.where(k == FULL, FULL * LANES, k * LANES + REM), REM)
        blk = jnp.concatenate([xT_v[g, pl.ds(r0, REM), :], xT_v[g, pl.ds(r1, REM), :]], axis=0)
        xN[k, pl.ds(pl.multiple_of(g * LANES, LANES), LANES), :] = blk.astype(F32).T

    def store_out_block(g, k):
        blk = outN[pl.ds(pl.multiple_of(g * LANES, LANES), LANES),
                   pl.ds(pl.multiple_of(k * LANES, LANES), LANES)].T.astype(BF16)
        r0 = pl.multiple_of(k * LANES, REM)
        r1 = pl.multiple_of(jnp.where(k == FULL, FULL * LANES, k * LANES + REM), REM)
        outT_v[g, pl.ds(r0, REM), :] = blk[:REM]
        outT_v[g, pl.ds(r1, REM), :] = blk[REM:]

    def layernorm_mod(xt, shift, scl):
        def tot(ts):
            acc = ts[FULL] * 0.5
            for t in range(FULL):
                acc = acc + ts[t]
            return jnp.sum(acc, axis=1, keepdims=True) / D
        m = tot(xt)
        v = tot([(t - m) * (t - m) for t in xt])
        mb = _rb(m)
        sd = _rb(jnp.sqrt(_rb(_rb(v) + 1e-5)))
        return [_rb(_rb(_rb(_rb(t - mb) / sd) * scl[j]) + shift[j]) for j, t in enumerate(xt)]

    def make_h(seg):
        sa = _tiles(par[0])
        ca1 = _tiles(par[1])
        for b in range(SEG // 8):
            r = pl.multiple_of(seg * SEG + b * 8, 8)
            ht = layernorm_mod([xN[t, pl.ds(r, 8), :] for t in range(NT)], sa, ca1)
            hs[b * 8:(b + 1) * 8, :] = jnp.concatenate(ht, axis=1)

    x_copy(0).wait()
    for k in range(NT):
        load_x_block(0, k)
    make_h(0)
    for g in range(1, NG):
        x_copy(g).wait()

    low = lane < REM
    tril = (lane & 7) <= sub

    def group_allreduce(x, op):
        for k in (1, 2, 4):
            up = pltpu.roll(x, k, 1)
            dn = pltpu.roll(x, LANES - k, 1)
            x = op(x, jnp.where((lane & k) != 0, up, dn))
        return x

    def wchunk(ref, t):
        n = H if t < FULL else NP
        return jnp.concatenate(
            [pltpu.bitcast(ref[t * H + j], BF16) for j in range(n)], axis=1)

    def stack(y, t):
        if t < FULL:
            parts = [y[b * 8:(b + 1) * 8, h * LANES:(h + 1) * LANES]
                     for b in range(NB) for h in range(H)]
        else:
            parts = []
            for b in range(NB):
                for p in range(NP):
                    v = y[b * 8:(b + 1) * 8, p * LANES:(p + 1) * LANES]
                    parts += [jnp.where(low, v, 0.0), jnp.where(low, 0.0, v)]
        return jnp.concatenate(parts, axis=0).astype(BF16)

    def finish_segment(seg, valid, best, besti):
        ga = _tiles(par[2])
        sb = _tiles(par[3])
        cb1 = _tiles(par[4])
        gb = _tiles(par[5])
        wrt = _tiles(par[6])
        for b in range(SEG // 8):
            r = pl.multiple_of(seg * SEG + b * 8, 8)
            at = _tiles(att[b * 8:(b + 1) * 8, :])
            x1 = [_rb(xN[t, pl.ds(r, 8), :] + _rb(ga[t] * _rb(at[t]))) for t in range(NT)]
            h2 = layernorm_mod(x1, sb, cb1)
            rr = functools.reduce(jnp.add, [h2[t] * wrt[t] for t in range(NT)])
            rr = _rb(jnp.broadcast_to(jnp.sum(rr, axis=1, keepdims=True), (8, LANES)))
            better = jnp.logical_and(rr > best, valid)
            best = jnp.where(better, rr, best)
            besti = jnp.where(better, sub + r, besti)
            h2s[0, pl.ds(r, 8), :] = jnp.concatenate(h2, axis=1)
            h2s[1, pl.ds(r, 8), :] = jnp.concatenate(x1, axis=1)
            outN[pl.ds(r, 8), :] = jnp.concatenate(
                [x1[t] + _rb(gb[t] * (h2[t] + h2[t] * 0.0)) for t in range(NT)], axis=1)
        return best, besti

    def softmax(sc_):
        prow = []
        for ib in range(NB):
            nj = NB if ib == 0 else ib + 1
            ts = [sc_[ib * 8:(ib + 1) * 8, jb * LANES:(jb + 1) * LANES] for jb in range(nj)]
            if ib > 0:
                ts[ib] = jnp.where(tril, ts[ib], -1e9)
            m = functools.reduce(jnp.maximum, ts)
            m = group_allreduce(m, jnp.maximum)
            es = [jnp.exp(t - m) for t in ts]
            l = group_allreduce(functools.reduce(jnp.add, es), jnp.add)
            inv = 1.0 / l
            ps = [e * inv for e in es] + [jnp.zeros((8, LANES), F32)] * (NB - nj)
            prow.append(jnp.concatenate(ps, axis=1))
        return jnp.concatenate(prow, axis=0)

    def step(s, carry):
        mem, best, besti = carry
        g = s // SPG
        k = s - g * SPG
        rows = jnp.concatenate([mem, hs[...]], axis=0)
        rt = _tiles(rows)

        def key_chunk(t):
            return stack(_dot(rows, wchunk(wa, t), _NN), t)

        def val_chunk(t):
            return stack(_dot(rows, wchunk(wb, t), _NN), t)

        k0 = key_chunk(0)
        load_x_block(jnp.minimum(g + 1, NG - 1), k)
        make_h(jnp.minimum(s + 1, NSEG - 1))
        k1 = key_chunk(1)
        sc_ = _dot(rt[0], k0, _NT)
        best, besti = finish_segment(jnp.maximum(s - 1, 0), s > 0, best, besti)
        k2 = key_chunk(2)
        sc_ = sc_ + _dot(rt[1], k1, _NT)
        store_out_block(jnp.maximum(g - 1, 0), k)
        k3 = key_chunk(3)
        sc_ = sc_ + _dot(rt[2], k2, _NT)
        u0 = val_chunk(0)
        sc_ = sc_ + _dot(rt[3], k3, _NT)
        u1 = val_chunk(1)
        p = softmax(sc_)
        u2 = val_chunk(2)
        u3 = val_chunk(3)
        outs = [_dot(p, u, _NN) for u in (u0, u1, u2, u3)]
        outs[FULL] = outs[FULL] + pltpu.roll(outs[FULL], REM, 1)
        mem = jnp.concatenate([o[0:M] for o in outs], axis=1)
        att[...] = jnp.concatenate([o[M:] for o in outs], axis=1)
        return mem, best, besti

    att[...] = jnp.zeros(att.shape, F32)
    mem0 = dup(mem0_ref[...].astype(F32))
    _, best, besti = lax.fori_loop(
        0, NSEG, step,
        (mem0, jnp.full((8, LANES), -jnp.inf, F32), jnp.zeros((8, LANES), jnp.int32)))
    best, besti = finish_segment(NSEG - 1, True, best, besti)

    for k in range(NT):
        store_out_block(NG - 1, k)

    top = jnp.max(best, axis=0, keepdims=True)
    cand = jnp.where(best == top, besti, S)
    idx = jnp.minimum(jnp.min(cand), S - 1)

    for cp in ffn_copies:
        cp.wait()
    h_sel = h2s[0, pl.ds(idx, 1), :]
    x_sel = h2s[1, pl.ds(idx, 1), :]
    hb = jnp.broadcast_to(h_sel[:, :D], (8, D)).astype(BF16)
    gt = _rb(_dot(hb, wg_v[...], _NN))
    up = _rb(_dot(hb, wu_v[...], _NN))
    act = _rb(_rb(gt * jax.nn.sigmoid(gt)) * up)
    y = _rb(_dot(act.astype(BF16), wd_v[...], _NT))
    y = _rb(y * _rb(jax.nn.sigmoid(top[:, 0:1])))
    hh = jnp.broadcast_to(h_sel, (8, NT * LANES))
    new = x_sel + _rb(par[5] * _rb(hh + _rb(hh * 0.0 + dup(y))))
    outN[pl.ds(idx, 1), :] = new[0:1]
    gsel = idx // LANES
    for k in range(NT):
        store_out_block(gsel, k)

    ocs = [pltpu.make_async_copy(outT_v.at[g], outT_hbm.at[:, g * LANES:(g + 1) * LANES], sem_o.at[g])
           for g in range(NG)]
    for cp in ocs:
        cp.start()
    for cp in ocs:
        cp.wait()


@functools.partial(jax.jit, static_argnames=("A_seg_len",))
def pallas_adaLN_cond__memory_aug_recurrent_mem_tr__moe_arch_mod__prompt_kernel(
    A_x, A_mem0, A_Wq, A_Wk, A_Wv, A_Wo, A_seg_len, B_x, B_w_r, B_w_gate, B_w_up, B_w_down, c, w_mod,
):
    del B_x
    _, S, D = A_x.shape
    _, H, E = A_Wq.shape
    M = A_mem0.shape[1]
    SEG = int(A_seg_len)
    FF = B_w_gate.shape[1]
    NG = S // LANES
    NT = D // LANES + 1
    NCT = (NT - 1) * H + H // 2

    anyspec = pl.BlockSpec(memory_space=pltpu.HBM)
    vspec = pl.BlockSpec(memory_space=pltpu.VMEM)
    vm = pltpu.VMEM
    outT = pl.pallas_call(
        functools.partial(_kernel, S=S, D=D, H=H, E=E, M=M, SEG=SEG),
        out_shape=jax.ShapeDtypeStruct((D, S), A_x.dtype),
        in_specs=[anyspec, vspec, anyspec, anyspec, anyspec, anyspec, vspec, anyspec, anyspec, anyspec,
                  vspec, anyspec],
        out_specs=anyspec,
        scratch_shapes=[
            vm((H // 2, D, E), U32), vm((H // 2, D, E), U32), vm((H // 2, D, E), U32),
            vm((H // 2, 2, D, E), BF16),
            vm((NCT, NT * LANES // 2, LANES), U32), vm((NCT, NT * LANES // 2, LANES), U32),
            vm(w_mod.shape, BF16),
            vm((NG, D, LANES), BF16),
            vm((NT, S, LANES), F32),
            vm((SEG, NT * LANES), F32),
            vm((2, S, NT * LANES), F32),
            vm((S, NT * LANES), F32),
            vm((NG, D, LANES), BF16),
            vm((D, FF), BF16), vm((D, FF), BF16), vm((D, FF), BF16),
            vm((7, 8, NT * LANES), F32),
            vm((SEG, NT * LANES), F32),
            pltpu.SemaphoreType.DMA((4, H // 2)),
            pltpu.SemaphoreType.DMA((NG,)),
            pltpu.SemaphoreType.DMA((NG,)),
            pltpu.SemaphoreType.DMA((4,)),
        ],
        compiler_params=pltpu.CompilerParams(vmem_limit_bytes=100 * 1024 * 1024),
        name="adaln_rmt_mod",
    )(jnp.swapaxes(A_x[0], 0, 1), A_mem0[0], A_Wq, A_Wk, A_Wv, jnp.swapaxes(A_Wo, 1, 2), B_w_r,
      B_w_gate, B_w_up, jnp.swapaxes(B_w_down, 0, 1), c, w_mod)
    return jnp.swapaxes(outT, 0, 1)[None]
```

```python
import functools

import jax
import jax.numpy as jnp
import numpy as np
from jax import lax
import jax.experimental.pallas as pl
import jax.experimental.pallas.tpu as pltpu

F32 = jnp.float32
BF16 = jnp.bfloat16
U32 = jnp.uint32

_NN = (((1,), (0,)), ((), ()))
_NT = (((1,), (1,)), ((), ()))

LANES = 128
GPI = 2


def _dot(a, b, dims):
    return lax.dot_general(a, b, dims, preferred_element_type=F32)


def _rb(x):
    return x.astype(BF16).astype(F32)


def _unpack(w):
    lo = pltpu.bitcast(w << 16, F32)
    hi = pltpu.bitcast(w & np.uint32(0xFFFF0000), F32)
    return lo, hi


def _pack(x):
    return pltpu.bitcast(x.astype(BF16), U32)


def _tiles(x):
    return [x[:, t * LANES:(t + 1) * LANES] for t in range(x.shape[1] // LANES)]


def _blk(x, i, j):
    return x[i * 8:(i + 1) * 8, j * LANES:(j + 1) * LANES]


def _kernel(xT_hbm, mem0_ref, wq_hbm, wk_hbm, wv_hbm, woT_hbm, wr_ref, wg_hbm, wu_hbm, wdT_hbm,
            c_ref, wmod_hbm, outT_hbm,
            bq, bk, bv, bo, wa, wb, wa2, wb2, wmod_v, xT_v, xN, hs, keep, outN, outT_v,
            wg_v, wu_v, wd_v, par, att, p_s, u_s, sem_w, sem_m,
            *, S, D, H, E, M, SEG):
    NG = S // LANES
    NSEG = S // SEG
    SPG = LANES // SEG
    L = M + SEG
    NB = L // 8
    NP = H // 2
    FULL = D // LANES
    DM = FULL * LANES
    REM = D - DM
    NT = FULL + 1
    scale = float(E) ** -0.5
    assert M == 8 and 8 * H == LANES and 2 * REM == LANES and NB <= NP and NG % GPI == 0

    wq32 = wq_hbm.bitcast(U32)
    wk32 = wk_hbm.bitcast(U32)
    wv32 = wv_hbm.bitcast(U32)

    def qk_copies(i):
        return (pltpu.make_async_copy(wq32.at[:, i, :], bq.at[i], sem_w.at[i]),
                pltpu.make_async_copy(wk32.at[:, i, :], bk.at[i], sem_w.at[i]))

    def vo_copies(i):
        return (pltpu.make_async_copy(woT_hbm.at[pl.ds(2 * i, 2)], bo.at[i], sem_w.at[i + 1]),
                pltpu.make_async_copy(wv32.at[:, i, :], bv.at[i], sem_w.at[i + 1]))

    x_early = range(1, GPI + 2)
    x_late = range(GPI + 2, NG)

    def x_copy(g):
        sem = sem_m.at[0 if g == 0 else (1 if g in x_early else 2)]
        return pltpu.make_async_copy(xT_hbm.at[:, g * LANES:(g + 1) * LANES], xT_v.at[g], sem)

    def out_copy(g):
        dst = outT_hbm.at[:, pl.ds(pl.multiple_of(g * LANES, LANES), LANES)]
        return pltpu.make_async_copy(outT_v.at[g], dst, sem_m.at[3])

    ffn_copies = (pltpu.make_async_copy(wg_hbm, wg_v, sem_m.at[4]),
                  pltpu.make_async_copy(wu_hbm, wu_v, sem_m.at[4]),
                  pltpu.make_async_copy(wdT_hbm, wd_v, sem_m.at[4]))
    mod_copy = pltpu.make_async_copy(wmod_hbm, wmod_v, sem_m.at[5])

    x_copy(0).start()
    for i in range(NP + 1):
        for cp in (qk_copies(i) if i < NP else ()) + (vo_copies(i - 1) if i else ()):
            cp.start()
    mod_copy.start()
    for g in x_early:
        x_copy(g).start()

    lane = lax.broadcasted_iota(jnp.int32, (8, LANES), 1)
    sub = lax.broadcasted_iota(jnp.int32, (8, LANES), 0)
    low = lane < REM
    tril = (lane & 7) <= sub
    pair_of_lane = lane // 16

    outN[0:LANES, :] = jnp.zeros((LANES, NT * LANES), F32)
    att[...] = jnp.zeros(att.shape, F32)
    par[...] = jnp.zeros(par.shape, F32)

    def load_x_block(g, k):
        if k < FULL:
            blk = xT_v[g, k * LANES:(k + 1) * LANES, :]
        else:
            blk = xT_v[g, DM:, :]
            blk = jnp.concatenate([blk, blk], axis=0)
        xN[k, pl.ds(pl.multiple_of(g * LANES, LANES), LANES), :] = blk.astype(F32).T

    def store_out_block(g, k):
        blk = outN[pl.ds(pl.multiple_of(g * LANES, LANES), LANES), k * LANES:(k + 1) * LANES].T
        if k < FULL:
            outT_v[g, k * LANES:(k + 1) * LANES, :] = blk.astype(BF16)
            return [blk[LANES - 8:]]
        outT_v[g, DM:, :] = blk[:REM].astype(BF16)
        return [blk[REM - 8:REM]]

    def layernorm(xt):
        def mean(ts):
            acc = ts[FULL] * 0.5
            for t in range(FULL):
                acc = acc + ts[t]
            return jnp.sum(acc, axis=1, keepdims=True) * (1.0 / D)
        m = mean(xt)
        v = mean([(t - m) * (t - m) for t in xt])
        mb = _rb(m)
        inv = 1.0 / _rb(jnp.sqrt(_rb(_rb(v) + 1e-5)))
        return [_rb(_rb(t - mb) * inv) for t in xt]

    def modulate(xt, shift, one_plus_scale):
        return [_rb(_rb(t * one_plus_scale[j]) + shift[j]) for j, t in enumerate(xt)]

    def make_h(seg):
        sa, ca1 = _tiles(par[0]), _tiles(par[1])
        done = []
        for b in range(SEG // 8):
            r = pl.multiple_of(seg * SEG + b * 8, 8)
            ht = modulate(layernorm([xN[t, pl.ds(r, 8), :] for t in range(NT)]), sa, ca1)
            hs[b * 8:(b + 1) * 8, :] = jnp.concatenate(ht, axis=1)
            done.append(ht)
        return done

    def finish_segment(seg, valid, best, besti):
        ga, sb, cb1, gb, wrt = (_tiles(par[j]) for j in range(2, 7))
        done = []
        for b in range(SEG // 8):
            r = pl.multiple_of(seg * SEG + b * 8, 8)
            at = _tiles(att[b * 8:(b + 1) * 8, :])
            at[FULL] = at[FULL] + pltpu.roll(at[FULL], REM, 1)
            x1 = [_rb(xN[t, pl.ds(r, 8), :] + _rb(ga[t] * _rb(at[t]))) for t in range(NT)]
            h2 = modulate(layernorm(x1), sb, cb1)
            rr = functools.reduce(jnp.add, [h2[t] * wrt[t] for t in range(NT)])
            rr = _rb(jnp.broadcast_to(jnp.sum(rr, axis=1, keepdims=True), (8, LANES)))
            better = jnp.logical_and(rr > best, valid)
            best = jnp.where(better, rr, best)
            besti = jnp.where(better, sub + r, besti)
            keep[0, pl.ds(r, 8), :] = jnp.concatenate(h2, axis=1)
            keep[1, pl.ds(r, 8), :] = jnp.concatenate(x1, axis=1)
            res = [x1[t] + _rb(gb[t] * (h2[t] + h2[t] * 0.0)) for t in range(NT)]
            outN[pl.ds(r, 8), :] = jnp.concatenate(res, axis=1)
            done.append(res + [best])
        return best, besti, done

    x_copy(0).wait()
    for k in range(NT):
        load_x_block(0, k)
    for b in range(SEG // 8):
        hs[b * 8:(b + 1) * 8, :] = jnp.concatenate(
            layernorm([xN[t, b * 8:(b + 1) * 8, :] for t in range(NT)]), axis=1)

    low_main = lax.broadcasted_iota(jnp.int32, (DM, LANES), 1) < REM
    low_rem = lax.broadcasted_iota(jnp.int32, (REM, LANES), 1) < REM

    def fuse(lhs_lo, lhs_hi, r_lo, r_hi, dst, i, mul):
        rem = jnp.concatenate([r_lo[DM:], r_hi[DM:]], axis=0)
        outs = []
        for j, (lhs, r) in enumerate(((lhs_lo, r_lo), (lhs_hi, r_hi))):
            o = _dot(lhs, jnp.concatenate([r[:DM], rem], axis=0), _NT)
            if mul != 1.0:
                o = o * mul
            for t in range(FULL):
                dst[t * H + 2 * i + j] = _pack(o[:DM, t * LANES:(t + 1) * LANES])
            outs.append(o)
        dst[FULL * H + i] = _pack(jnp.where(low_main, outs[0][:DM, DM:], outs[1][:DM, DM:]))
        tail_lo = jnp.concatenate([outs[0][DM:, :DM], jnp.where(low_rem, outs[0][DM:, DM:], 0.0)], axis=1)
        tail_hi = jnp.concatenate([outs[1][DM:, :DM], jnp.where(low_rem, 0.0, outs[1][DM:, DM:])], axis=1)
        return jnp.concatenate([tail_lo, tail_hi], axis=0)

    def fuse_qk(i):
        q_lo, q_hi = _unpack(bq[i])
        k_lo, k_hi = _unpack(bk[i])
        wa2[i] = _pack(fuse(k_lo, k_hi, q_lo.astype(BF16), q_hi.astype(BF16), wa, i, scale).T)

    def fuse_vo(i):
        v_lo, v_hi = _unpack(bv[i])
        wb2[i] = _pack(fuse(v_lo, v_hi, bo[i, 0], bo[i, 1], wb, i, 1.0))

    def fuse_body(i, carry):
        for cp in vo_copies(i) + qk_copies(i + 1):
            cp.wait()
        fuse_qk(i + 1)
        fuse_vo(i)
        return carry

    for cp in qk_copies(0):
        cp.wait()
    fuse_qk(0)
    lax.fori_loop(0, NP - 1, fuse_body, 0)
    for cp in vo_copies(NP - 1):
        cp.wait()
    fuse_vo(NP - 1)
    mod_copy.wait()
    for g in x_late:
        x_copy(g).start()

    def dup(v):
        return jnp.concatenate([v, v[:, DM:]], axis=1)

    cv = jnp.broadcast_to(c_ref[...].astype(F32), (8, D))
    mod = _rb(_dot((cv * jax.nn.sigmoid(cv)).astype(BF16), wmod_v[...], _NN))
    for j in range(6):
        v = mod[:, j * D:(j + 1) * D]
        par[j] = dup(_rb(1.0 + v) if j in (1, 4) else v)
    wr = jnp.broadcast_to(wr_ref[...].astype(F32).reshape(1, D), (8, D))
    par[6] = jnp.concatenate([wr, jnp.zeros((8, REM), F32)], axis=1)
    for b in range(SEG // 8):
        hs[b * 8:(b + 1) * 8, :] = jnp.concatenate(
            modulate(_tiles(hs[b * 8:(b + 1) * 8, :]), _tiles(par[0]), _tiles(par[1])), axis=1)
    for g in x_early:
        x_copy(g).wait()
    load_x_block(1, 0)

    def needed(ib, jb):
        return ib == 0 or jb <= ib

    def visible(jb):
        return [ib for ib in range(NB) if needed(ib, jb)]

    def take(x, ibs):
        return jnp.concatenate([x[ib * 8:(ib + 1) * 8] for ib in ibs], axis=0)

    def spread(r, jb):
        ibs = visible(jb)
        zero = jnp.zeros((8, r.shape[1]), F32)
        return jnp.concatenate(
            [r[ibs.index(ib) * 8:(ibs.index(ib) + 1) * 8] if ib in ibs else zero for ib in range(NB)], axis=0)

    def per_head(x, op):
        for k in (1, 2, 4):
            up = pltpu.roll(x, k, 1)
            dn = pltpu.roll(x, LANES - k, 1)
            x = op(x, jnp.where((lane & k) != 0, up, dn))
        return x

    def softmax(sc, sx):
        prob = []
        for ib in range(NB):
            ts = []
            for jb in range(NB):
                if not needed(ib, jb):
                    continue
                e = _blk(sx[(-jb) % NP], ib, 0)
                for m in range(1, NP):
                    e = jnp.where(pair_of_lane == m, _blk(sx[(m - jb) % NP], ib, 0), e)
                if jb:
                    e = pltpu.roll(e, LANES - 16 * jb, 1)
                t = _blk(sc, ib, jb) + e
                ts.append(jnp.where(tril, t, -1e9) if (ib and jb == ib) else t)
            m = per_head(functools.reduce(jnp.maximum, ts), jnp.maximum)
            es = [jnp.exp(t - m) for t in ts]
            inv = 1.0 / per_head(functools.reduce(jnp.add, es), jnp.add)
            prob.append([e * inv for e in es])
        zero = jnp.zeros((8, LANES), F32)
        p = jnp.concatenate([jnp.concatenate(r + [zero] * (NB - len(r)), axis=1) for r in prob], axis=0)
        rolled = [[pltpu.roll(t, 16 * jb, 1) if jb else t for jb, t in enumerate(r)] for r in prob]
        pp = []
        for q in range(NP):
            blocks = []
            for r in rolled:
                e = r[0] if len(r) == NB else jnp.where(pair_of_lane == q, r[0], 0.0)
                for jb in range(1, len(r)):
                    e = jnp.where(pair_of_lane == (q + jb) % NP, r[jb], e)
                blocks.append(e)
            pp.append(jnp.concatenate(blocks, axis=0))
        return p, pp

    def attend(p, us):
        first = jnp.concatenate([jnp.concatenate([u[jb] for u in us], axis=1) for jb in (0, 1)], axis=0)
        acc = _dot(p[:, :2 * LANES], first, _NN)
        acc = [acc[ib * 8:(ib + 1) * 8] for ib in range(NB)]
        for jb in range(2, NB):
            ibs = visible(jb)
            r = _dot(take(p[:, jb * LANES:(jb + 1) * LANES], ibs),
                     jnp.concatenate([u[jb] for u in us], axis=1), _NN)
            for n, ib in enumerate(ibs):
                acc[ib] = acc[ib] + r[n * 8:(n + 1) * 8]
        return jnp.concatenate(acc, axis=0)

    def key_blocks(u):
        return [u[jb * LANES:(jb + 1) * LANES] for jb in range(NB)]

    def wcols(ref, c0, n):
        return jnp.concatenate([pltpu.bitcast(ref[c0 + j], BF16) for j in range(n)], axis=1)

    def stack(ys):
        out = []
        for jb in range(NB):
            parts = [y[jb * 8:(jb + 1) * 8] for y in ys]
            if len(ys) == NP:
                parts = [w for v in parts for w in (jnp.where(low, v, 0.0), jnp.where(low, 0.0, v))]
            out.append(jnp.concatenate(parts, axis=0).astype(BF16))
        return out

    def step(g, k, mem, part, p_prev, v_prev, best, besti):
        s = g * SPG + k
        ht = _tiles(hs[...])
        rt = [jnp.concatenate([mem[t], ht[t]], axis=0) for t in range(FULL)]
        rows = jnp.concatenate(rt, axis=1)

        def cols(ref, c0, n, after=None):
            lhs = rows
            if after is not None:
                bits = functools.reduce(jnp.bitwise_or, [pltpu.bitcast(a, U32) for a in after])
                bits = bits & pltpu.bitcast(par[7, :, 0:LANES], U32)
                first = pltpu.bitcast(pltpu.bitcast(mem[0], U32) | bits, F32)
                lhs = jnp.concatenate([jnp.concatenate([first, ht[0]], axis=0)] + rt[1:], axis=1)
            return _tiles(_dot(lhs, wcols(ref, c0, n), _NN))

        k0 = stack(cols(wa, 0, H))
        o3 = part + attend(p_prev, [key_blocks(v_prev)])
        att[:, DM:] = o3[M:]
        q3 = jnp.concatenate([o3[0:M] + pltpu.roll(o3[0:M], REM, 1), ht[FULL]], axis=0)
        qt = rt + [q3]

        slots = [jnp.concatenate([jnp.where(low, _blk(q3, jb, 0), 0.0),
                                  jnp.where(low, 0.0, _blk(q3, jb, 0))], axis=0).astype(BF16)
                 for jb in range(NB)]
        zslot = jnp.zeros((16, LANES), BF16)
        gt = [jnp.concatenate([slots[(m - q) % NP] if (m - q) % NP < NB else zslot for m in range(NP)], axis=0)
              for q in range(NP)]

        def score(t, ks):
            parts = [_dot(qt[t], jnp.concatenate(ks[:2], axis=0), _NT)]
            parts += [spread(_dot(take(qt[t], visible(jb)), ks[jb], _NT), jb) for jb in range(2, NB - 1)]
            return jnp.concatenate(parts, axis=1)

        def score_rem(q0):
            return [_dot(rq[q], gt[q], _NT) for q in range(q0, q0 + NP // 2)]

        load_x_block(jnp.minimum(g + 1 + (k + 1) // SPG, NG - 1), (k + 1) % SPG)
        d1 = make_h(jnp.minimum(s + 1, NSEG - 1))
        ya = cols(wa, H, NP)
        sc = score(0, k0)
        k1 = stack(ya + cols(wa, H + NP, NP, d1[0]))
        rq = _tiles(_dot(jnp.concatenate(qt, axis=1), wcols(wa2, 0, NP), _NN))
        sc = sc + score(1, k1)
        ya = cols(wa, 2 * H, NP, d1[1])
        sx = score_rem(0)
        k2 = stack(ya + cols(wa, 2 * H + NP, NP, d1[2]))
        sx = sx + score_rem(NP // 2)
        k3 = stack(cols(wa, 3 * H, NP, d1[3]))
        sc = sc + score(2, k2)
        ya = cols(wb, 0, 7)
        sc = sc + score(3, k3)
        ya = ya + cols(wb, 7, 5)
        last = _dot(take(jnp.concatenate(qt, axis=1), visible(NB - 1)),
                    jnp.concatenate([ks[NB - 1] for ks in (k0, k1, k2, k3)], axis=1), _NT)
        sc = jnp.concatenate([sc, spread(last, NB - 1)], axis=1)
        v0 = stack(ya + cols(wb, 12, H - 12))
        best, besti, d2 = finish_segment(jnp.maximum(s - 1, 0), s > 0, best, besti)
        d3 = store_out_block(jnp.maximum(g - 1, 0), k)
        p, pp = softmax(sc, sx)
        v1 = stack(cols(wb, H, NP, d2[0]) + cols(wb, H + NP, NP, d2[1]))
        v2 = stack(cols(wb, 2 * H, NP, d2[2]) + cols(wb, 2 * H + NP, NP, d2[3]))
        o01 = attend(p, (v0, v1))
        ph = jnp.concatenate([_dot(pp[q], gt[q], _NN) for q in range(NP)], axis=1)
        o2 = attend(p, (v2,))
        ya = cols(wb, 3 * H, 3)
        orem = _dot(ph, jnp.concatenate([pltpu.bitcast(wb2[q], BF16) for q in range(NP)], axis=0), _NN)
        v3 = jnp.concatenate(stack(ya + cols(wb, 3 * H + 3, NP - 3, d3)), axis=0)
        o = jnp.concatenate([o01, o2], axis=1) + orem[:, :DM]
        att[:, :DM] = o[M:]
        return _tiles(o[0:M]), orem[:, DM:], p, v3, best, besti

    def body(it, carry):
        mem, best, besti = carry
        g0 = it * GPI

        @pl.when(it == 1)
        def _():
            for g in x_late:
                x_copy(g).wait()
            for cp in ffn_copies:
                cp.start()

        for j in range(GPI):
            @pl.when(g0 - 2 - j >= 0)
            def _():
                out_copy(g0 - 2 - j).start()

        part = p_s[:, NB * LANES:]
        p = p_s[:, :NB * LANES]
        v3 = pltpu.bitcast(u_s[...], BF16)
        for j in range(GPI):
            for k in range(SPG):
                mem, part, p, v3, best, besti = step(g0 + j, k, list(mem), part, p, v3, best, besti)
        p_s[:, NB * LANES:] = part
        p_s[:, :NB * LANES] = p
        u_s[...] = pltpu.bitcast(v3, U32)
        return tuple(mem), best, besti

    mem0 = _tiles(jnp.concatenate([mem0_ref[...].astype(F32), jnp.zeros((M, REM), F32)], axis=1))
    p_s[...] = jnp.zeros(p_s.shape, F32)
    p_s[0:M, NB * LANES:] = mem0[FULL]
    u_s[...] = jnp.zeros(u_s.shape, U32)
    _, best, besti = lax.fori_loop(
        0, NG // GPI, body,
        (tuple(mem0[:FULL]), jnp.full((8, LANES), -jnp.inf, F32), jnp.zeros((8, LANES), jnp.int32)))
    for j in range(GPI):
        out_copy(NG - 2 - j).start()
    o3 = p_s[:, NB * LANES:] + _dot(p_s[:, :NB * LANES], pltpu.bitcast(u_s[...], BF16), _NN)
    att[:, DM:] = o3[M:]
    best, besti, _ = finish_segment(NSEG - 1, True, best, besti)
    for k in range(NT):
        store_out_block(NG - 1, k)
    out_copy(NG - 1).start()

    top = jnp.max(best, axis=0, keepdims=True)
    idx = jnp.minimum(jnp.min(jnp.where(best == top, besti, S)), S - 1)

    for cp in ffn_copies:
        cp.wait()
    h_sel = keep[0, pl.ds(idx, 1), :]
    x_sel = keep[1, pl.ds(idx, 1), :]
    hb = jnp.broadcast_to(h_sel[:, :D], (8, D)).astype(BF16)
    gate = _rb(_dot(hb, wg_v[...], _NN))
    up = _rb(_dot(hb, wu_v[...], _NN))
    act = _rb(gate * jax.nn.sigmoid(gate)) * up
    y = _rb(_dot(act.astype(BF16), wd_v[...], _NT))
    y = _rb(y * _rb(jax.nn.sigmoid(top[:, 0:1])))
    hh = jnp.broadcast_to(h_sel, (8, NT * LANES))
    new = x_sel + _rb(par[5] * _rb(hh + _rb(hh * 0.0 + dup(y))))
    outN[pl.ds(idx, 1), :] = new[0:1]

    gsel = idx // LANES
    for g in range(NG):
        out_copy(g).wait()
    for k in range(NT):
        store_out_block(gsel, k)
    out_copy(gsel).start()
    out_copy(gsel).wait()


@functools.partial(jax.jit, static_argnames=("A_seg_len",))
def pallas_adaLN_cond__memory_aug_recurrent_mem_tr__moe_arch_mod__prompt_kernel(
    A_x, A_mem0, A_Wq, A_Wk, A_Wv, A_Wo, A_seg_len, B_x, B_w_r, B_w_gate, B_w_up, B_w_down, c, w_mod,
):
    del B_x
    _, S, D = A_x.shape
    _, H, E = A_Wq.shape
    M = A_mem0.shape[1]
    SEG = int(A_seg_len)
    FF = B_w_gate.shape[1]
    L = M + SEG
    NG = S // LANES
    NP = H // 2
    FULL = D // LANES
    DP = (FULL + 1) * LANES

    hbm = pl.BlockSpec(memory_space=pltpu.HBM)
    vmem = pl.BlockSpec(memory_space=pltpu.VMEM)
    buf = pltpu.VMEM
    outT = pl.pallas_call(
        functools.partial(_kernel, S=S, D=D, H=H, E=E, M=M, SEG=SEG),
        out_shape=jax.ShapeDtypeStruct((D, S), A_x.dtype),
        in_specs=[hbm, vmem, hbm, hbm, hbm, hbm, vmem, hbm, hbm, hbm, vmem, hbm],
        out_specs=hbm,
        scratch_shapes=[
            buf((NP, D, E), U32), buf((NP, D, E), U32), buf((NP, D, E), U32),
            buf((NP, 2, D, E), BF16),
            buf((FULL * H + NP, FULL * LANES // 2, LANES), U32),
            buf((FULL * H + NP, FULL * LANES // 2, LANES), U32),
            buf((NP, DP // 2, LANES), U32),
            buf((NP, LANES // 2, DP), U32),
            buf(w_mod.shape, BF16),
            buf((NG, D, LANES), BF16),
            buf((FULL + 1, S, LANES), F32),
            buf((SEG, DP), F32),
            buf((2, S, DP), F32),
            buf((S, DP), F32),
            buf((NG, D, LANES), BF16),
            buf((D, FF), BF16), buf((D, FF), BF16), buf((D, FF), BF16),
            buf((8, 8, DP), F32),
            buf((SEG, DP), F32),
            buf((L, L * H + LANES), F32),
            buf((L * H // 2, LANES), U32),
            pltpu.SemaphoreType.DMA((NP + 1,)),
            pltpu.SemaphoreType.DMA((6,)),
        ],
        compiler_params=pltpu.CompilerParams(vmem_limit_bytes=100 * 1024 * 1024),
        name="adaln_rmt_mod",
    )(jnp.swapaxes(A_x[0], 0, 1), A_mem0[0], A_Wq, A_Wk, A_Wv, jnp.swapaxes(A_Wo, 1, 2), B_w_r,
      B_w_gate, B_w_up, jnp.swapaxes(B_w_down, 0, 1), c, w_mod)
    return jnp.swapaxes(outT, 0, 1)[None]
```

```python
import functools

import jax
import jax.numpy as jnp
import numpy as np
from jax import lax
import jax.experimental.pallas as pl
import jax.experimental.pallas.tpu as pltpu

F32 = jnp.float32
BF16 = jnp.bfloat16
U32 = jnp.uint32

_NN = (((1,), (0,)), ((), ()))
_NT = (((1,), (1,)), ((), ()))

LANES = 128
GPI = 2


def _dot(a, b, dims):
    return lax.dot_general(a, b, dims, preferred_element_type=F32)


def _rb(x):
    return x.astype(BF16).astype(F32)


def _unpack(w):
    lo = pltpu.bitcast(w << 16, F32)
    hi = pltpu.bitcast(w & np.uint32(0xFFFF0000), F32)
    return lo, hi


def _pack(x):
    return pltpu.bitcast(x.astype(BF16), U32)


def _tiles(x):
    return [x[:, t * LANES:(t + 1) * LANES] for t in range(x.shape[1] // LANES)]


def _blk(x, i, j):
    return x[i * 8:(i + 1) * 8, j * LANES:(j + 1) * LANES]


def _kernel(xT_hbm, mem0_ref, wq_hbm, wk_hbm, wv_hbm, woT_hbm, wr_ref, wg_hbm, wu_hbm, wdT_hbm,
            c_ref, wmod_hbm, outT_hbm,
            bq, bk, bv, bo, wa, wb, wa2, wb2, wmod_v, xT_v, xN, hs, keep, outN, outT_v,
            wg_v, wu_v, wd_v, par, att, p_s, u_s, sem_w, sem_m,
            *, S, D, H, E, M, SEG):
    NG = S // LANES
    NSEG = S // SEG
    SPG = LANES // SEG
    L = M + SEG
    NB = L // 8
    NP = H // 2
    FULL = D // LANES
    DM = FULL * LANES
    REM = D - DM
    NT = FULL + 1
    scale = float(E) ** -0.5
    assert M == 8 and 8 * H == LANES and 2 * REM == LANES and NB <= NP and NG % GPI == 0

    wq32 = wq_hbm.bitcast(U32)
    wk32 = wk_hbm.bitcast(U32)
    wv32 = wv_hbm.bitcast(U32)

    def qk_copies(i):
        return (pltpu.make_async_copy(wq32.at[:, i, :], bq.at[i], sem_w.at[i]),
                pltpu.make_async_copy(wk32.at[:, i, :], bk.at[i], sem_w.at[i]))

    def vo_copies(i):
        return (pltpu.make_async_copy(woT_hbm.at[pl.ds(2 * i, 2)], bo.at[i], sem_w.at[i + 1]),
                pltpu.make_async_copy(wv32.at[:, i, :], bv.at[i], sem_w.at[i + 1]))

    x_early = range(1, GPI + 2)
    x_late = range(GPI + 2, NG)

    def x_copy(g):
        sem = sem_m.at[0 if g == 0 else (1 if g in x_early else 2)]
        return pltpu.make_async_copy(xT_hbm.at[:, g * LANES:(g + 1) * LANES], xT_v.at[g], sem)

    def out_copy(g):
        dst = outT_hbm.at[:, pl.ds(pl.multiple_of(g * LANES, LANES), LANES)]
        return pltpu.make_async_copy(outT_v.at[g], dst, sem_m.at[3])

    ffn_copies = (pltpu.make_async_copy(wg_hbm, wg_v, sem_m.at[4]),
                  pltpu.make_async_copy(wu_hbm, wu_v, sem_m.at[4]),
                  pltpu.make_async_copy(wdT_hbm, wd_v, sem_m.at[4]))
    mod_copy = pltpu.make_async_copy(wmod_hbm, wmod_v, sem_m.at[5])

    x_copy(0).start()
    for i in range(NP + 1):
        for cp in (qk_copies(i) if i < NP else ()) + (vo_copies(i - 1) if i else ()):
            cp.start()
    mod_copy.start()
    for g in x_early:
        x_copy(g).start()

    lane = lax.broadcasted_iota(jnp.int32, (8, LANES), 1)
    sub = lax.broadcasted_iota(jnp.int32, (8, LANES), 0)
    low = lane < REM
    tril = (lane & 7) <= sub
    pair_of_lane = lane // 16

    outN[0:LANES, :] = jnp.zeros((LANES, NT * LANES), F32)
    att[...] = jnp.zeros(att.shape, F32)
    par[...] = jnp.zeros(par.shape, F32)

    def load_x_block(g, k):
        if k < FULL:
            blk = xT_v[g, k * LANES:(k + 1) * LANES, :]
        else:
            blk = xT_v[g, DM:, :]
            blk = jnp.concatenate([blk, blk], axis=0)
        xN[k, pl.ds(pl.multiple_of(g * LANES, LANES), LANES), :] = blk.astype(F32).T

    def store_out_block(g, k):
        blk = outN[pl.ds(pl.multiple_of(g * LANES, LANES), LANES), k * LANES:(k + 1) * LANES].T
        if k < FULL:
            outT_v[g, k * LANES:(k + 1) * LANES, :] = blk.astype(BF16)
            return [blk[LANES - 8:]]
        outT_v[g, DM:, :] = blk[:REM].astype(BF16)
        return [blk[REM - 8:REM]]

    def layernorm(xt):
        def mean(ts):
            acc = ts[FULL] * 0.5
            for t in range(FULL):
                acc = acc + ts[t]
            return jnp.sum(acc, axis=1, keepdims=True) * (1.0 / D)
        m = mean(xt)
        v = mean([(t - m) * (t - m) for t in xt])
        mb = _rb(m)
        inv = 1.0 / _rb(jnp.sqrt(_rb(_rb(v) + 1e-5)))
        return [_rb(_rb(t - mb) * inv) for t in xt]

    def modulate(xt, shift, one_plus_scale):
        return [_rb(_rb(t * one_plus_scale[j]) + shift[j]) for j, t in enumerate(xt)]

    def make_h(seg):
        sa, ca1 = _tiles(par[0]), _tiles(par[1])
        done = []
        for b in range(SEG // 8):
            r = pl.multiple_of(seg * SEG + b * 8, 8)
            ht = modulate(layernorm([xN[t, pl.ds(r, 8), :] for t in range(NT)]), sa, ca1)
            hs[b * 8:(b + 1) * 8, :] = jnp.concatenate(ht, axis=1)
            done.append(ht)
        return done

    def finish_segment(seg, valid, best, besti):
        ga, sb, cb1, gb, wrt = (_tiles(par[j]) for j in range(2, 7))
        done = []
        for b in range(SEG // 8):
            r = pl.multiple_of(seg * SEG + b * 8, 8)
            at = _tiles(att[b * 8:(b + 1) * 8, :])
            at[FULL] = at[FULL] + pltpu.roll(at[FULL], REM, 1)
            x1 = [_rb(xN[t, pl.ds(r, 8), :] + _rb(ga[t] * _rb(at[t]))) for t in range(NT)]
            h2 = modulate(layernorm(x1), sb, cb1)
            rr = functools.reduce(jnp.add, [h2[t] * wrt[t] for t in range(NT)])
            rr = _rb(jnp.broadcast_to(jnp.sum(rr, axis=1, keepdims=True), (8, LANES)))
            better = jnp.logical_and(rr > best, valid)
            best = jnp.where(better, rr, best)
            besti = jnp.where(better, sub + r, besti)
            keep[0, pl.ds(r, 8), :] = jnp.concatenate(h2, axis=1)
            keep[1, pl.ds(r, 8), :] = jnp.concatenate(x1, axis=1)
            res = [x1[t] + _rb(gb[t] * (h2[t] + h2[t] * 0.0)) for t in range(NT)]
            outN[pl.ds(r, 8), :] = jnp.concatenate(res, axis=1)
            done.append(res + [best])
        return best, besti, done

    x_copy(0).wait()
    for k in range(NT):
        load_x_block(0, k)
    for b in range(SEG // 8):
        hs[b * 8:(b + 1) * 8, :] = jnp.concatenate(
            layernorm([xN[t, b * 8:(b + 1) * 8, :] for t in range(NT)]), axis=1)

    low_main = lax.broadcasted_iota(jnp.int32, (DM, LANES), 1) < REM
    low_rem = lax.broadcasted_iota(jnp.int32, (REM, LANES), 1) < REM

    def fuse(lhs_lo, lhs_hi, r_lo, r_hi, dst, i, mul):
        rem = jnp.concatenate([r_lo[DM:], r_hi[DM:]], axis=0)
        outs = []
        for j, (lhs, r) in enumerate(((lhs_lo, r_lo), (lhs_hi, r_hi))):
            o = _dot(lhs, jnp.concatenate([r[:DM], rem], axis=0), _NT)
            if mul != 1.0:
                o = o * mul
            for t in range(FULL):
                dst[t * H + 2 * i + j] = _pack(o[:DM, t * LANES:(t + 1) * LANES])
            outs.append(o)
        dst[FULL * H + i] = _pack(jnp.where(low_main, outs[0][:DM, DM:], outs[1][:DM, DM:]))
        tail_lo = jnp.concatenate([outs[0][DM:, :DM], jnp.where(low_rem, outs[0][DM:, DM:], 0.0)], axis=1)
        tail_hi = jnp.concatenate([outs[1][DM:, :DM], jnp.where(low_rem, 0.0, outs[1][DM:, DM:])], axis=1)
        return jnp.concatenate([tail_lo, tail_hi], axis=0)

    def fuse_qk(i):
        q_lo, q_hi = _unpack(bq[i])
        k_lo, k_hi = _unpack(bk[i])
        wa2[i] = _pack(fuse(k_lo, k_hi, q_lo.astype(BF16), q_hi.astype(BF16), wa, i, scale).T)

    def fuse_vo(i):
        v_lo, v_hi = _unpack(bv[i])
        wb2[i] = _pack(fuse(v_lo, v_hi, bo[i, 0], bo[i, 1], wb, i, 1.0))

    def fuse_body(i, carry):
        for cp in vo_copies(i) + qk_copies(i + 1):
            cp.wait()
        fuse_qk(i + 1)
        fuse_vo(i)
        return carry

    for cp in qk_copies(0):
        cp.wait()
    fuse_qk(0)
    lax.fori_loop(0, NP - 1, fuse_body, 0)
    for cp in vo_copies(NP - 1):
        cp.wait()
    fuse_vo(NP - 1)
    mod_copy.wait()
    for g in x_late:
        x_copy(g).start()

    def dup(v):
        return jnp.concatenate([v, v[:, DM:]], axis=1)

    cv = jnp.broadcast_to(c_ref[...].astype(F32), (8, D))
    mod = _rb(_dot((cv * jax.nn.sigmoid(cv)).astype(BF16), wmod_v[...], _NN))
    for j in range(6):
        v = mod[:, j * D:(j + 1) * D]
        par[j] = dup(_rb(1.0 + v) if j in (1, 4) else v)
    wr = jnp.broadcast_to(wr_ref[...].astype(F32).reshape(1, D), (8, D))
    par[6] = jnp.concatenate([wr, jnp.zeros((8, REM), F32)], axis=1)
    for b in range(SEG // 8):
        hs[b * 8:(b + 1) * 8, :] = jnp.concatenate(
            modulate(_tiles(hs[b * 8:(b + 1) * 8, :]), _tiles(par[0]), _tiles(par[1])), axis=1)
    for g in x_early:
        x_copy(g).wait()
    load_x_block(1, 0)

    def needed(ib, jb):
        return ib == 0 or jb <= ib

    def visible(jb):
        return [ib for ib in range(NB) if needed(ib, jb)]

    def take(x, ibs):
        return jnp.concatenate([x[ib * 8:(ib + 1) * 8] for ib in ibs], axis=0)

    def spread(r, jb):
        ibs = visible(jb)
        zero = jnp.zeros((8, r.shape[1]), F32)
        return jnp.concatenate(
            [r[ibs.index(ib) * 8:(ibs.index(ib) + 1) * 8] if ib in ibs else zero for ib in range(NB)], axis=0)

    def per_head(x, op):
        for k in (1, 2, 4):
            up = pltpu.roll(x, k, 1)
            dn = pltpu.roll(x, LANES - k, 1)
            x = op(x, jnp.where((lane & k) != 0, up, dn))
        return x

    def softmax(sc, sx):
        prob = []
        for ib in range(NB):
            ts = []
            for jb in range(NB):
                if not needed(ib, jb):
                    continue
                e = _blk(sx[(-jb) % NP], ib, 0)
                for m in range(1, NP):
                    e = jnp.where(pair_of_lane == m, _blk(sx[(m - jb) % NP], ib, 0), e)
                if jb:
                    e = pltpu.roll(e, LANES - 16 * jb, 1)
                t = _blk(sc, ib, jb) + e
                ts.append(jnp.where(tril, t, -1e9) if (ib and jb == ib) else t)
            m = per_head(functools.reduce(jnp.maximum, ts), jnp.maximum)
            es = [jnp.exp(t - m) for t in ts]
            inv = 1.0 / per_head(functools.reduce(jnp.add, es), jnp.add)
            prob.append([e * inv for e in es])
        zero = jnp.zeros((8, LANES), F32)
        p = jnp.concatenate([jnp.concatenate(r + [zero] * (NB - len(r)), axis=1) for r in prob], axis=0)
        rolled = [[pltpu.roll(t, 16 * jb, 1) if jb else t for jb, t in enumerate(r)] for r in prob]
        pp = []
        for q in range(NP):
            blocks = []
            for r in rolled:
                e = r[0] if len(r) == NB else jnp.where(pair_of_lane == q, r[0], 0.0)
                for jb in range(1, len(r)):
                    e = jnp.where(pair_of_lane == (q + jb) % NP, r[jb], e)
                blocks.append(e)
            pp.append(jnp.concatenate(blocks, axis=0))
        return p, pp

    def attend(p, us):
        first = jnp.concatenate([jnp.concatenate([u[jb] for u in us], axis=1) for jb in (0, 1)], axis=0)
        acc = _dot(p[:, :2 * LANES], first, _NN)
        acc = [acc[ib * 8:(ib + 1) * 8] for ib in range(NB)]
        for jb in range(2, NB):
            ibs = visible(jb)
            r = _dot(take(p[:, jb * LANES:(jb + 1) * LANES], ibs),
                     jnp.concatenate([u[jb] for u in us], axis=1), _NN)
            for n, ib in enumerate(ibs):
                acc[ib] = acc[ib] + r[n * 8:(n + 1) * 8]
        return jnp.concatenate(acc, axis=0)

    def key_blocks(u):
        return [u[jb * LANES:(jb + 1) * LANES] for jb in range(NB)]

    def wcols(ref, c0, n):
        return jnp.concatenate([pltpu.bitcast(ref[c0 + j], BF16) for j in range(n)], axis=1)

    def stack(ys):
        out = []
        for jb in range(NB):
            parts = [y[jb * 8:(jb + 1) * 8] for y in ys]
            if len(ys) == NP:
                parts = [w for v in parts for w in (jnp.where(low, v, 0.0), jnp.where(low, 0.0, v))]
            out.append(jnp.concatenate(parts, axis=0).astype(BF16))
        return out

    def step(g, k, mem, part, p_prev, v_prev, best, besti):
        s = g * SPG + k
        ht = _tiles(hs[...])
        rt = [jnp.concatenate([mem[t], ht[t]], axis=0) for t in range(FULL)]
        rows = jnp.concatenate(rt, axis=1)

        def cols(ref, c0, n, after=None):
            lhs = rows
            if after is not None:
                bits = functools.reduce(jnp.bitwise_or, [pltpu.bitcast(a, U32) for a in after])
                bits = bits & pltpu.bitcast(par[7, :, 0:LANES], U32)
                first = pltpu.bitcast(pltpu.bitcast(mem[0], U32) | bits, F32)
                lhs = jnp.concatenate([jnp.concatenate([first, ht[0]], axis=0)] + rt[1:], axis=1)
            return _tiles(_dot(lhs, wcols(ref, c0, n), _NN))

        k0 = stack(cols(wa, 0, H))
        o3 = part + attend(p_prev, [key_blocks(v_prev)])
        att[:, DM:] = o3[M:]
        q3 = jnp.concatenate([o3[0:M] + pltpu.roll(o3[0:M], REM, 1), ht[FULL]], axis=0)
        qt = rt + [q3]

        slots = [jnp.concatenate([jnp.where(low, _blk(q3, jb, 0), 0.0),
                                  jnp.where(low, 0.0, _blk(q3, jb, 0))], axis=0).astype(BF16)
                 for jb in range(NB)]
        zslot = jnp.zeros((16, LANES), BF16)
        gt = [jnp.concatenate([slots[(m - q) % NP] if (m - q) % NP < NB else zslot for m in range(NP)], axis=0)
              for q in range(NP)]

        def score(t, ks):
            parts = [_dot(qt[t], jnp.concatenate(ks[:2], axis=0), _NT)]
            parts += [spread(_dot(take(qt[t], visible(jb)), ks[jb], _NT), jb) for jb in range(2, NB - 1)]
            return jnp.concatenate(parts, axis=1)

        def score_rem(q0):
            return [_dot(rq[q], gt[q], _NT) for q in range(q0, q0 + NP // 2)]

        load_x_block(jnp.minimum(g + 1 + (k + 1) // SPG, NG - 1), (k + 1) % SPG)
        d1 = make_h(jnp.minimum(s + 1, NSEG - 1))
        ya = cols(wa, H, NP)
        sc = score(0, k0)
        k1 = stack(ya + cols(wa, H + NP, NP, d1[0]))
        rq = _tiles(_dot(jnp.concatenate(qt, axis=1), wcols(wa2, 0, NP), _NN))
        sc = sc + score(1, k1)
        ya = cols(wa, 2 * H, NP, d1[1])
        sx = score_rem(0)
        k2 = stack(ya + cols(wa, 2 * H + NP, NP, d1[2]))
        sx = sx + score_rem(NP // 2)
        k3 = stack(cols(wa, 3 * H, NP, d1[3]))
        sc = sc + score(2, k2)
        ya = cols(wb, 0, 7)
        sc = sc + score(3, k3)
        ya = ya + cols(wb, 7, 5)
        last = _dot(take(jnp.concatenate(qt, axis=1), visible(NB - 1)),
                    jnp.concatenate([ks[NB - 1] for ks in (k0, k1, k2, k3)], axis=1), _NT)
        sc = jnp.concatenate([sc, spread(last, NB - 1)], axis=1)
        v0 = stack(ya + cols(wb, 12, H - 12))
        best, besti, d2 = finish_segment(jnp.maximum(s - 1, 0), s > 0, best, besti)
        d3 = store_out_block(jnp.maximum(g - 1, 0), k)
        p, pp = softmax(sc, sx)
        v1 = stack(cols(wb, H, NP, d2[0]) + cols(wb, H + NP, NP, d2[1]))
        v2 = stack(cols(wb, 2 * H, NP, d2[2]) + cols(wb, 2 * H + NP, NP, d2[3]))
        ya = cols(wb, 3 * H, 2)
        o01 = attend(p, (v0, v1))
        ph = jnp.concatenate([_dot(pp[q], gt[q], _NN) for q in range(NP)], axis=1)
        o2 = attend(p, (v2,))
        ya = ya + cols(wb, 3 * H + 2, 1)
        orem = _dot(ph, jnp.concatenate([pltpu.bitcast(wb2[q], BF16) for q in range(NP)], axis=0), _NN)
        v3 = jnp.concatenate(stack(ya + cols(wb, 3 * H + 3, NP - 3, d3)), axis=0)
        o = jnp.concatenate([o01, o2], axis=1) + orem[:, :DM]
        att[:, :DM] = o[M:]
        return _tiles(o[0:M]), orem[:, DM:], p, v3, best, besti

    def body(it, carry):
        mem, best, besti = carry
        g0 = it * GPI

        @pl.when(it == 1)
        def _():
            for g in x_late:
                x_copy(g).wait()
            for cp in ffn_copies:
                cp.start()

        for j in range(GPI):
            @pl.when(g0 - 2 - j >= 0)
            def _():
                out_copy(g0 - 2 - j).start()

        part = p_s[:, NB * LANES:]
        p = p_s[:, :NB * LANES]
        v3 = pltpu.bitcast(u_s[...], BF16)
        for j in range(GPI):
            for k in range(SPG):
                mem, part, p, v3, best, besti = step(g0 + j, k, list(mem), part, p, v3, best, besti)
        p_s[:, NB * LANES:] = part
        p_s[:, :NB * LANES] = p
        u_s[...] = pltpu.bitcast(v3, U32)
        return tuple(mem), best, besti

    mem0 = _tiles(jnp.concatenate([mem0_ref[...].astype(F32), jnp.zeros((M, REM), F32)], axis=1))
    p_s[...] = jnp.zeros(p_s.shape, F32)
    p_s[0:M, NB * LANES:] = mem0[FULL]
    u_s[...] = jnp.zeros(u_s.shape, U32)
    _, best, besti = lax.fori_loop(
        0, NG // GPI, body,
        (tuple(mem0[:FULL]), jnp.full((8, LANES), -jnp.inf, F32), jnp.zeros((8, LANES), jnp.int32)))
    for j in range(GPI):
        out_copy(NG - 2 - j).start()

    def argmax(best, besti):
        top = jnp.max(best, axis=0, keepdims=True)
        return top, jnp.minimum(jnp.min(jnp.where(best == top, besti, S)), S - 1)

    def ffn(idx):
        hb = jnp.broadcast_to(keep[0, pl.ds(idx, 1), :][:, :D], (8, D)).astype(BF16)
        gate = _rb(_dot(hb, wg_v[...], _NN))
        up = _rb(_dot(hb, wu_v[...], _NN))
        act = _rb(gate * jax.nn.sigmoid(gate)) * up
        par[7] = dup(_rb(_dot(act.astype(BF16), wd_v[...], _NT)))

    for cp in ffn_copies:
        cp.wait()
    _, lead = argmax(best, besti)
    o3 = p_s[:, NB * LANES:] + _dot(p_s[:, :NB * LANES], pltpu.bitcast(u_s[...], BF16), _NN)
    att[:, DM:] = o3[M:]
    ffn(lead)
    best, besti, _ = finish_segment(NSEG - 1, True, best, besti)
    for k in range(NT):
        store_out_block(NG - 1, k)
    top, idx = argmax(best, besti)
    out_copy(NG - 1).start()

    @pl.when(idx != lead)
    def _():
        ffn(idx)

    y = _rb(par[7] * _rb(jax.nn.sigmoid(top[:, 0:1])))
    hh = jnp.broadcast_to(keep[0, pl.ds(idx, 1), :], (8, NT * LANES))
    new = keep[1, pl.ds(idx, 1), :] + _rb(par[5] * _rb(hh + _rb(hh * 0.0 + y)))
    outN[pl.ds(idx, 1), :] = new[0:1]

    gsel = idx // LANES
    for g in range(NG):
        out_copy(g).wait()
    for k in range(NT):
        store_out_block(gsel, k)
    out_copy(gsel).start()
    out_copy(gsel).wait()


@functools.partial(jax.jit, static_argnames=("A_seg_len",))
def pallas_adaLN_cond__memory_aug_recurrent_mem_tr__moe_arch_mod__prompt_kernel(
    A_x, A_mem0, A_Wq, A_Wk, A_Wv, A_Wo, A_seg_len, B_x, B_w_r, B_w_gate, B_w_up, B_w_down, c, w_mod,
):
    del B_x
    _, S, D = A_x.shape
    _, H, E = A_Wq.shape
    M = A_mem0.shape[1]
    SEG = int(A_seg_len)
    FF = B_w_gate.shape[1]
    L = M + SEG
    NG = S // LANES
    NP = H // 2
    FULL = D // LANES
    DP = (FULL + 1) * LANES

    hbm = pl.BlockSpec(memory_space=pltpu.HBM)
    vmem = pl.BlockSpec(memory_space=pltpu.VMEM)
    buf = pltpu.VMEM
    outT = pl.pallas_call(
        functools.partial(_kernel, S=S, D=D, H=H, E=E, M=M, SEG=SEG),
        out_shape=jax.ShapeDtypeStruct((D, S), A_x.dtype),
        in_specs=[hbm, vmem, hbm, hbm, hbm, hbm, vmem, hbm, hbm, hbm, vmem, hbm],
        out_specs=hbm,
        scratch_shapes=[
            buf((NP, D, E), U32), buf((NP, D, E), U32), buf((NP, D, E), U32),
            buf((NP, 2, D, E), BF16),
            buf((FULL * H + NP, FULL * LANES // 2, LANES), U32),
            buf((FULL * H + NP, FULL * LANES // 2, LANES), U32),
            buf((NP, DP // 2, LANES), U32),
            buf((NP, LANES // 2, DP), U32),
            buf(w_mod.shape, BF16),
            buf((NG, D, LANES), BF16),
            buf((FULL + 1, S, LANES), F32),
            buf((SEG, DP), F32),
            buf((2, S, DP), F32),
            buf((S, DP), F32),
            buf((NG, D, LANES), BF16),
            buf((D, FF), BF16), buf((D, FF), BF16), buf((D, FF), BF16),
            buf((8, 8, DP), F32),
            buf((SEG, DP), F32),
            buf((L, L * H + LANES), F32),
            buf((L * H // 2, LANES), U32),
            pltpu.SemaphoreType.DMA((NP + 1,)),
            pltpu.SemaphoreType.DMA((6,)),
        ],
        compiler_params=pltpu.CompilerParams(vmem_limit_bytes=100 * 1024 * 1024),
        name="adaln_rmt_mod",
    )(jnp.swapaxes(A_x[0], 0, 1), A_mem0[0], A_Wq, A_Wk, A_Wv, jnp.swapaxes(A_Wo, 1, 2), B_w_r,
      B_w_gate, B_w_up, jnp.swapaxes(B_w_down, 0, 1), c, w_mod)
    return jnp.swapaxes(outT, 0, 1)[None]
```
